```python
import jax
import jax.numpy as jnp

def _softmax(x, axis=-1):
    return jax.nn.softmax(x, axis=axis)

def _gelu(x):
    return jax.nn.gelu(x, approximate=True)

def _silu(x):
    return jax.nn.silu(x)

def _sigmoid(x):
    return jax.nn.sigmoid(x)

def _layernorm(x, axis=-1, eps=1e-05):
    m = jnp.mean(x, axis=axis, keepdims=True)
    v = jnp.var(x, axis=axis, keepdims=True)
    return (x - m) / jnp.sqrt(v + eps)

def _scatter_add(tgt, idx, src, axis=0):
    return tgt.at[idx].add(src)

def _segment_sum(src, seg, n):
    return jax.ops.segment_sum(src, seg, n)

class _Rng:

    def __init__(self, key):
        self._k = key

    def _next(self):
        self._k, sub = jax.random.split(self._k)
        return sub

    def normal(self, shape):
        return jax.random.normal(self._next(), shape, dtype=jnp.bfloat16)

    def randint(self, lo, hi, shape):
        return jax.random.randint(self._next(), shape, lo, hi, dtype=jnp.int32)

    def uniform(self, shape, lo=0.0, hi=1.0):
        return jax.random.uniform(self._next(), shape, jnp.bfloat16, lo, hi)

    def permutation(self, n):
        return jax.random.permutation(self._next(), n)
kernel_name = 'interleave_layers__memory_aug_recurrent_mem_tr__linear_kernel_hedgehog__prompt'

def setup_inputs():
    _rng = _Rng(jax.random.key(int.from_bytes(__import__("os").urandom(4), "little")))
    _w = lambda a: (lambda t: t.astype(jnp.bfloat16) if jnp.issubdtype(t.dtype, jnp.floating) else t)(jnp.asarray(a))

    def _A_setup():
        B, S, Dm = (1, 2048, 640)
        H, Dh = (32, 192)
        M, seg = (8, 32)
        seg = min(seg, S)
        S = S // seg * seg
        return {'x': _w((lambda *s: _rng.normal(s) * 0.05)(B, S, Dm)), 'mem0': _w((lambda *s: _rng.normal(s) * 0.05)(B, M, Dm)), 'Wq': _w((lambda *s: _rng.normal(s) * 0.05)(Dm, H, Dh) * Dm ** (-0.5)), 'Wk': _w((lambda *s: _rng.normal(s) * 0.05)(Dm, H, Dh) * Dm ** (-0.5)), 'Wv': _w((lambda *s: _rng.normal(s) * 0.05)(Dm, H, Dh) * Dm ** (-0.5)), 'Wo': _w((lambda *s: _rng.normal(s) * 0.05)(H, Dh, Dm) * (H * Dh) ** (-0.5)), 'seg_len': seg}
    _A_in = _A_setup()

    def _B_setup():
        B, S, D, H = (1, 2048, 640, 32)
        Dh = D // H
        return {'x': _w((lambda *s: _rng.normal(s) * 0.05)(B, S, D)), 'wqkv': _w((lambda *s: _rng.normal(s) * 0.05)(D, 3 * D)), 'w_phi': _w((lambda *s: _rng.normal(s) * 0.05)(H, Dh, Dh) * Dh ** (-0.5)), 'wo': _w((lambda *s: _rng.normal(s) * 0.05)(D, D))}
    _B_in = _B_setup()
    return {'A_x': _A_in['x'], 'A_mem0': _A_in['mem0'], 'A_Wq': _A_in['Wq'], 'A_Wk': _A_in['Wk'], 'A_Wv': _A_in['Wv'], 'A_Wo': _A_in['Wo'], 'A_seg_len': _A_in['seg_len'], 'B_x': _B_in['x'], 'B_wqkv': _B_in['wqkv'], 'B_w_phi': _B_in['w_phi'], 'B_wo': _B_in['wo']}

def reference(A_x, A_mem0, A_Wq, A_Wk, A_Wv, A_Wo, A_seg_len, B_x, B_wqkv, B_w_phi, B_wo):

    def _A_ref(x, mem0, Wq, Wk, Wv, Wo, seg_len):
        B, S, Dm = x.shape
        H, Dh = (Wq.shape[1], Wq.shape[2])
        M = mem0.shape[1]
        scale = Dh ** (-0.5)
        n_seg = S // seg_len
        L = M + seg_len
        idx = jnp.arange(L)
        mask = (idx[:, None] < M) | (idx[:, None] >= idx[None, :])
        mem = mem0
        outs = []
        for s in range(n_seg):
            xs = x[:, s * seg_len:(s + 1) * seg_len, :].copy()
            h = jnp.concatenate([mem, xs], axis=1)
            q = jnp.einsum('btd,dhe->bhte', h, Wq)
            k = jnp.einsum('btd,dhe->bhte', h, Wk)
            v = jnp.einsum('btd,dhe->bhte', h, Wv)
            scores = jnp.einsum('bhqe,bhke->bhqk', q, k) * scale
            scores = jnp.where(mask[None, None], scores, -1000000000.0)
            p = _softmax(scores, axis=-1)
            o = jnp.einsum('bhqk,bhke->bhqe', p, v)
            o = jnp.einsum('bhte,hed->btd', o, Wo)
            mem = o[:, :M, :].copy()
            outs.append(o[:, M:, :])
        return jnp.concatenate(outs, axis=1)

    def _B_ref(x, wqkv, w_phi, wo):
        B, S, D = x.shape
        H = 32
        Dh = D // H
        qkv = (lambda x, *d: x.transpose(*d))((x @ wqkv).reshape(B, S, 3, H, Dh), 2, 0, 3, 1, 4)
        q, k, v = (qkv[0], qkv[1], qkv[2])
        pq = jnp.einsum('bhsd,hdf->bhsf', q, w_phi)
        pk = jnp.einsum('bhsd,hdf->bhsf', k, w_phi)
        phi_q = jnp.concatenate([_softmax(pq, axis=-1), _softmax(-pq, axis=-1)], axis=-1)
        phi_k = jnp.concatenate([_softmax(pk, axis=-1), _softmax(-pk, axis=-1)], axis=-1)
        kv = jnp.einsum('bhsf,bhsd->bhfd', phi_k, v)
        z = jnp.einsum('bhsf->bhf', phi_k)
        num = jnp.einsum('bhqf,bhfd->bhqd', phi_q, kv)
        den = jnp.einsum('bhqf,bhf->bhq', phi_q, z)[..., None] + 1e-06
        o = num / den
        return (lambda x, *d: x.transpose(*d))(o, 0, 2, 1, 3).reshape(B, S, D) @ wo
    x = A_x
    x = x + _A_ref(_layernorm(x, axis=-1), A_mem0, A_Wq, A_Wk, A_Wv, A_Wo, A_seg_len)
    x = x + _B_ref(_layernorm(x, axis=-1), B_wqkv, B_w_phi, B_wo)
    x = x + _A_ref(_layernorm(x, axis=-1), A_mem0, A_Wq, A_Wk, A_Wv, A_Wo, A_seg_len)
    x = x + _B_ref(_layernorm(x, axis=-1), B_wqkv, B_w_phi, B_wo)
    return x
```

```python
import functools

import jax
import jax.numpy as jnp
from jax import lax
from jax.experimental import pallas as pl
from jax.experimental.pallas import tpu as pltpu

F32 = jnp.float32
BF16 = jnp.bfloat16
U32 = jnp.uint32

B_HEADS = 32
GROUP = 8
CHUNK = 512

_NT = (((1,), (1,)), ((), ()))
_TN = (((0,), (0,)), ((), ()))


def _dot(a, b):
    return jnp.dot(a, b, preferred_element_type=F32)


def _dot_nt(a, b):
    return lax.dot_general(a, b, _NT, preferred_element_type=F32)


def _dot_tn(a, b):
    return lax.dot_general(a, b, _TN, preferred_element_type=F32)


def _pack(w):
    return pltpu.bitcast(w, U32)


def _unpack(w):
    return pltpu.bitcast(w, BF16)


def _layernorm(x):
    m = jnp.mean(x, axis=-1, keepdims=True)
    c = x - m
    v = jnp.mean(c * c, axis=-1, keepdims=True)
    return c * lax.rsqrt(v + 1e-5)


def _iota(shape, dim):
    return lax.broadcasted_iota(jnp.int32, shape, dim)


def _feature_map(p, nf):
    rows = [p[f * GROUP:(f + 1) * GROUP] for f in range(nf)]
    hi = functools.reduce(jnp.maximum, rows)
    lo = functools.reduce(jnp.minimum, rows)
    ep = [jnp.exp(r - hi) for r in rows]
    en = [jnp.exp(lo - r) for r in rows]
    ip = 1.0 / functools.reduce(jnp.add, ep)
    im = 1.0 / functools.reduce(jnp.add, en)
    return jnp.concatenate([e * ip for e in ep] + [e * im for e in en], axis=0)


def _kernel(x_hbm, mem0_ref, wq_hbm, wk_hbm, wv_hbm, wo_hbm, bqkv_hbm, wphi_ref, bwo_hbm,
            out_hbm,
            xres, wqkv_s, wo_s, xnb, bq_s, bkv_s, bwo_s, h_s, kv_s, kvm_s, out_s, osem,
            *, seg, heads, dh):
    S, D = xres.shape
    M = mem0_ref.shape[0]
    L = M + seg
    n_seg = S // seg
    n_pair = heads // 2
    PW = 2 * dh
    bd = D // B_HEADS
    n_group = B_HEADS // GROUP
    GW = GROUP * bd
    n_chunk = S // CHUNK
    scale = dh ** -0.5

    def prologue(x_st, wt_st, wo_st, bqkv_st, bwo_st, sem, wsem):
        x_cp = pltpu.make_async_copy(x_hbm, x_st, sem.at[0])
        bqkv_cp = pltpu.make_async_copy(bqkv_hbm, bqkv_st, sem.at[1])
        bwo_cp = pltpu.make_async_copy(bwo_hbm, bwo_st, sem.at[2])

        def w_cp(j, p):
            rows = pl.ds(pl.multiple_of(p * PW, PW), PW)
            if j == 3:
                return pltpu.make_async_copy(wo_hbm.at[rows], wo_st.at[p], wsem.at[3, p])
            src = (wq_hbm, wk_hbm, wv_hbm)[j]
            return pltpu.make_async_copy(src.at[rows], wt_st.at[j, p], wsem.at[j, p])

        bqkv_cp.start()
        bwo_cp.start()
        x_cp.start()

        def start(p, c):
            for j in range(4):
                w_cp(j, p).start()
            return c

        lax.fori_loop(0, n_pair, start, 0)

        col = _iota((B_HEADS, D), 1) - bd * _iota((B_HEADS, D), 0)
        phi_t = jnp.zeros((bd, D), F32)
        for d in range(bd):
            sel = jnp.where(col == d, 1.0, 0.0).astype(BF16)
            phi_t = phi_t + _dot(wphi_ref[d], sel)
        bqkv_cp.wait()
        bwo_cp.wait()
        for g in range(n_group):
            off = _iota((GROUP, D), 1) - bd * (_iota((GROUP, D), 0) + g * GROUP)
            own = jnp.logical_and(off >= 0, off < bd)
            p_phi = jnp.concatenate(
                [jnp.where(own, phi_t[f:f + 1], 0.0) for f in range(bd)], axis=0).astype(BF16)
            p_id = jnp.concatenate(
                [jnp.where(off == f, 1.0, 0.0) for f in range(bd)], axis=0).astype(BF16)
            bq_s[g] = _dot_nt(p_phi, bqkv_st[:, 0:D]).astype(BF16)
            bkv_s[g, 0:GW] = _dot_nt(p_phi, bqkv_st[:, D:2 * D]).astype(BF16)
            bkv_s[g, GW:2 * GW] = _dot_nt(p_id, bqkv_st[:, 2 * D:3 * D]).astype(BF16)
            bwo_s[g * GW:(g + 1) * GW] = _dot(p_id, bwo_st[...]).astype(BF16)

        x_cp.wait()

        def widen(i, c):
            rows = pl.ds(pl.multiple_of(i * 128, 128), 128)
            xres[rows] = x_st[rows].astype(F32)
            return c

        lax.fori_loop(0, S // 128, widen, 0)

        def relayout(p, c):
            for j in range(3):
                w_cp(j, p).wait()
                wqkv_s[p, :, j * PW:(j + 1) * PW] = _pack(wt_st[j, p].T)
            w_cp(3, p).wait()
            wo_s[p] = _pack(wo_st[p])
            return c

        lax.fori_loop(0, n_pair, relayout, 0)

    pl.run_scoped(
        prologue,
        pltpu.VMEM((S, D), BF16),
        pltpu.VMEM((3, n_pair, PW, D), BF16),
        pltpu.VMEM((n_pair, PW, D), BF16),
        pltpu.VMEM((D, 3 * D), BF16),
        pltpu.VMEM((D, D), BF16),
        pltpu.SemaphoreType.DMA((3,)),
        pltpu.SemaphoreType.DMA((4, n_pair)),
    )

    def seg_rows(s):
        return pl.ds(pl.multiple_of(s * seg, seg), seg)

    def block_diag(t):
        first = _iota((L, PW), 1) < dh
        return jnp.concatenate(
            [jnp.where(first, t, 0.0), jnp.where(first, 0.0, t)], axis=0).astype(BF16)

    def a_step(s, c):
        h = h_s[...]
        qi = _iota((L, 2 * L), 0)
        lane = _iota((L, 2 * L), 1)
        head_a = lane < L
        kj = jnp.where(head_a, lane, lane - L)
        visible = jnp.logical_or(qi < M, qi >= kj)

        def project(p):
            qkv = _dot(h, _unpack(wqkv_s[p]))
            return qkv[:, 0:PW], block_diag(qkv[:, PW:2 * PW]), block_diag(qkv[:, 2 * PW:])

        def probs(q, k):
            sc = jnp.where(visible, _dot_nt(q, k) * scale, -1e9)
            ma = jnp.max(jnp.where(head_a, sc, -jnp.inf), axis=-1, keepdims=True)
            mb = jnp.max(jnp.where(head_a, -jnp.inf, sc), axis=-1, keepdims=True)
            e = jnp.exp(sc - jnp.where(head_a, ma, mb))
            la = jnp.sum(jnp.where(head_a, e, 0.0), axis=-1, keepdims=True)
            lb = jnp.sum(jnp.where(head_a, 0.0, e), axis=-1, keepdims=True)
            return e / jnp.where(head_a, la, lb)

        prev = seg_rows(jnp.maximum(s - 1, 0))
        xnb[prev] = _layernorm(xres[prev]).astype(BF16)
        x_next = _layernorm(xres[seg_rows(jnp.minimum(s + 1, n_seg - 1))])

        lag_s, lag_v, lag_o = 1, 2, 6
        qkv, pr, o = {}, {}, {}
        acc = None
        for t in range(n_pair + lag_o):
            if t < n_pair:
                qkv[t] = project(t)
            if 0 <= t - lag_s < n_pair:
                p = t - lag_s
                pr[p] = probs(qkv[p][0], qkv[p][1])
            if 0 <= t - lag_v < n_pair:
                p = t - lag_v
                o[p] = _dot(pr.pop(p), qkv.pop(p)[2])
            if 0 <= t - lag_o < n_pair:
                p = t - lag_o
                y = _dot(o.pop(p), _unpack(wo_s[p]))
                acc = y if acc is None else acc + y

        h_s[0:M] = acc[0:M]
        h_s[M:L] = x_next
        cur = seg_rows(s)
        xres[cur] = xres[cur] + acc[M:L]
        return c

    def layer_a():
        h_s[0:M] = mem0_ref[...].astype(F32)
        h_s[M:L] = _layernorm(xres[0:seg])
        lax.fori_loop(0, n_seg, a_step, 0)
        xnb[S - seg:S] = _layernorm(xres[S - seg:S]).astype(BF16)

    def chunk_rows(c):
        return pl.ds(pl.multiple_of(c * CHUNK, CHUNK), CHUNK)

    def b_keys(c, carry):
        xn = xnb[chunk_rows(c)]
        for g in range(n_group):
            kv = _dot_nt(bkv_s[g], xn)
            phi = _feature_map(kv[0:GW], bd).astype(BF16)
            v1 = jnp.concatenate([kv[GW:2 * GW], jnp.ones((2 * GROUP, CHUNK), F32)], axis=0)
            kv_s[g] += _dot_nt(v1.astype(BF16), phi)
        return carry

    def out_cp(c):
        return pltpu.make_async_copy(out_s.at[chunk_rows(c)], out_hbm.at[chunk_rows(c)], osem.at[c])

    def b_queries(c, last):
        rows = chunk_rows(c)
        xn = xnb[rows]
        heads_out = []
        for g in range(n_group):
            phi = _feature_map(_dot_nt(bq_s[g], xn), bd).astype(BF16)
            nd = _dot(kvm_s[g], phi)
            inv = 1.0 / (nd[GW:GW + GROUP] + 1e-6)
            heads_out += [nd[d * GROUP:(d + 1) * GROUP] * inv for d in range(bd)]
        o_t = jnp.concatenate(heads_out, axis=0).astype(BF16)
        y = xres[rows] + _dot_tn(o_t, bwo_s[...])
        xres[rows] = y
        out_s[rows] = y.astype(BF16)

        @pl.when(last)
        def _():
            out_cp(c).start()

    def layer_b(last):
        kv_s[...] = jnp.zeros(kv_s.shape, F32)
        lax.fori_loop(0, n_chunk, b_keys, 0)
        shape = kv_s.shape[1:]
        same_head = (_iota(shape, 0) % GROUP) == (_iota(shape, 1) % GROUP)
        for g in range(n_group):
            kvm_s[g] = jnp.where(same_head, kv_s[g], 0.0).astype(BF16)

        def body(c, carry):
            b_queries(c, last)
            return carry

        lax.fori_loop(0, n_chunk, body, 0)

    def layer_pair(i, c):
        layer_a()
        layer_b(i == 1)
        return c

    lax.fori_loop(0, 2, layer_pair, 0)
    for c in range(n_chunk):
        out_cp(c).wait()


@functools.partial(jax.jit, static_argnames=("A_seg_len",))
def pallas_interleave_layers__memory_aug_recurrent_mem_tr__linear_kernel_hedgehog__prompt_kernel(
    A_x: jax.Array,
    A_mem0: jax.Array,
    A_Wq: jax.Array,
    A_Wk: jax.Array,
    A_Wv: jax.Array,
    A_Wo: jax.Array,
    A_seg_len: int,
    B_x: jax.Array,
    B_wqkv: jax.Array,
    B_w_phi: jax.Array,
    B_wo: jax.Array,
):
    del B_x
    batch, S, D = A_x.shape
    _, H, dh = A_Wq.shape
    M = A_mem0.shape[1]
    seg = int(A_seg_len)
    assert batch == 1 and S % seg == 0 and S % CHUNK == 0 and H % 2 == 0
    GW = GROUP * (D // B_HEADS)
    n_group = B_HEADS // GROUP

    def head_major(w):
        return jnp.transpose(w, (1, 2, 0)).reshape(H * dh, D)

    hbm = pl.BlockSpec(memory_space=pl.ANY)
    vmem = pl.BlockSpec(memory_space=pltpu.VMEM)
    out = pl.pallas_call(
        functools.partial(_kernel, seg=seg, heads=H, dh=dh),
        out_shape=jax.ShapeDtypeStruct((S, D), A_x.dtype),
        in_specs=[hbm, vmem, hbm, hbm, hbm, hbm, hbm, vmem, hbm],
        out_specs=hbm,
        scratch_shapes=[
            pltpu.VMEM((S, D), F32),
            pltpu.VMEM((H // 2, D // 2, 6 * dh), U32),
            pltpu.VMEM((H // 2, dh, D), U32),
            pltpu.VMEM((S, D), BF16),
            pltpu.VMEM((n_group, GW, D), BF16),
            pltpu.VMEM((n_group, 2 * GW, D), BF16),
            pltpu.VMEM((D, D), BF16),
            pltpu.VMEM((M + seg, D), F32),
            pltpu.VMEM((n_group, GW + 2 * GROUP, 2 * GW), F32),
            pltpu.VMEM((n_group, GW + 2 * GROUP, 2 * GW), BF16),
            pltpu.VMEM((S, D), BF16),
            pltpu.SemaphoreType.DMA((S // CHUNK,)),
        ],
        compiler_params=pltpu.CompilerParams(vmem_limit_bytes=120 * 1024 * 1024),
    )(
        A_x.reshape(S, D),
        A_mem0.reshape(M, D),
        head_major(A_Wq),
        head_major(A_Wk),
        head_major(A_Wv),
        A_Wo.reshape(H * dh, D),
        B_wqkv,
        jnp.transpose(B_w_phi, (1, 2, 0)),
        B_wo,
    )
    return out.reshape(A_x.shape)
```

```python
import functools

import jax
import jax.numpy as jnp
from jax import lax
from jax.experimental import pallas as pl
from jax.experimental.pallas import tpu as pltpu

F32 = jnp.float32
BF16 = jnp.bfloat16
U32 = jnp.uint32

SUB = 8
B_HEADS = 32
GROUP = 2
SLAB = 8
UNROLL = 4
AHEAD = 7 * 128
IN_FLIGHT = 3
CHUNK = 512
OUT_CHUNK = 1024
OUT_SUB = 256

_NT = (((1,), (1,)), ((), ()))
_TN = (((0,), (0,)), ((), ()))


def _dot(a, b):
    return jnp.dot(a, b, preferred_element_type=F32)


def _dot_nt(a, b):
    return lax.dot_general(a, b, _NT, preferred_element_type=F32)


def _dot_tn(a, b):
    return lax.dot_general(a, b, _TN, preferred_element_type=F32)


def _pack(w):
    return pltpu.bitcast(w, U32)


def _unpack(w):
    return pltpu.bitcast(w, BF16)


def _layernorm(x):
    x = x.astype(F32)
    m = jnp.mean(x, axis=-1, keepdims=True)
    c = x - m
    v = jnp.mean(c * c, axis=-1, keepdims=True)
    return c * lax.rsqrt(v + 1e-5)


def _iota(shape, dim):
    return lax.broadcasted_iota(jnp.int32, shape, dim)


def _over_features(op, rows):
    r = functools.reduce(op, rows)
    shift = SUB // 2
    while shift >= GROUP:
        r = op(r, pltpu.roll(r, shift, 0))
        shift //= 2
    return r


def _feature_map(p):
    rows = [p[i:i + SUB] for i in range(0, p.shape[0], SUB)]
    hi = _over_features(jnp.maximum, rows)
    lo = _over_features(jnp.minimum, rows)
    ep = [jnp.exp(r - hi) for r in rows]
    en = [jnp.exp(lo - r) for r in rows]
    ip = 1.0 / _over_features(jnp.add, ep)
    im = 1.0 / _over_features(jnp.add, en)
    return jnp.concatenate([e * ip for e in ep] + [e * im for e in en], axis=0).astype(BF16)


def _kernel(x_hbm, mem0_hbm, wq_hbm, wk_hbm, wv_hbm, wo_hbm, bqkv_hbm, wphi_hbm, bwo_hbm,
            out_hbm,
            xres, wqkv_s, wo_s, ahead_s, xa_s, xnb, bw_s, bwo_s, v_s, phiq_s, kv_s, kvm_s, h_s,
            w_in, xa_in, mem0_in, bqkv_in, wphi_in, bwo_in, phi_s, wsem, sem, osem,
            *, heads, dh):
    n_seg, seg, D = xres.shape
    S = n_seg * seg
    M = mem0_in.shape[0]
    L = M + seg
    n_pair = heads // 2
    PW = 2 * dh
    bd = D // B_HEADS
    GW = GROUP * bd
    SW = SLAB * bd
    n_group = B_HEADS // GROUP
    n_slab = B_HEADS // SLAB
    per_slab = SLAB // GROUP
    scale = dh ** -0.5

    xa_cp = pltpu.make_async_copy(x_hbm.at[:, 0:SUB], xa_in, sem.at[0])
    wphi_cp = pltpu.make_async_copy(wphi_hbm, wphi_in, sem.at[1])
    mem0_cp = pltpu.make_async_copy(mem0_hbm, mem0_in, sem.at[2])
    x_cp = pltpu.make_async_copy(x_hbm, xres, sem.at[3])
    bqkv_cp = pltpu.make_async_copy(bqkv_hbm, bqkv_in, sem.at[4])
    bwo_cp = pltpu.make_async_copy(bwo_hbm, bwo_in, sem.at[5])

    def w_cp(j, p):
        src = (wq_hbm, wk_hbm, wv_hbm, wo_hbm)[j]
        return pltpu.make_async_copy(src.at[p], w_in.at[p, j], wsem.at[p, j])

    def fetch(p):
        for j in range(4):
            w_cp(j, p).start()

    def begin():
        wphi_cp.start()
        xa_cp.start()
        fetch(0)
        mem0_cp.start()
        xnb[0:UNROLL] = jnp.zeros((UNROLL,) + xnb.shape[1:], U32)
        wphi_cp.wait()
        col = _iota((B_HEADS, D), 1) - bd * _iota((B_HEADS, D), 0)
        phi_t = jnp.zeros((bd, D), F32)
        for d in range(bd):
            phi_t = phi_t + _dot(wphi_in[d], jnp.where(col == d, 1.0, 0.0).astype(BF16))
        row = _iota((SW, 128), 0) % GW
        spread = jnp.where(row // GROUP == _iota((SW, 128), 1), 1.0, 0.0)[:, 0:bd]
        phi_s[...] = _dot(spread, phi_t)
        xa_cp.wait()
        for p in range(1, IN_FLIGHT):
            fetch(p)
        xa = xa_in[...].astype(F32).reshape(n_seg * SUB, D)
        xa_s[...] = _pack(_layernorm(xa).astype(BF16))

    def arrive(p):
        for j in range(4):
            w_cp(j, p).wait()

    def prefetch(p, first):
        @pl.when(jnp.logical_and(first, p + IN_FLIGHT < n_pair))
        def _():
            fetch(p + IN_FLIGHT)

        for at, cp in zip((2, 6, 10), (x_cp, bqkv_cp, bwo_cp)):
            pl.when(jnp.logical_and(first, p == at))(cp.start)

    def prepare_b():
        for cp in (mem0_cp, x_cp, bqkv_cp, bwo_cp):
            cp.wait()
        for t in range(n_slab):
            c0 = t * SW // 128 * 128
            c1 = -(-(t + 1) * SW // 128) * 128
            r = _iota((SW, c1 - c0), 0)
            head = t * SLAB + r // GW * GROUP + r % GROUP
            off = _iota((SW, c1 - c0), 1) + c0 - bd * head
            own = jnp.logical_and(off >= 0, off < bd)
            p_phi = jnp.where(own, phi_s[:, c0:c1], 0.0).astype(BF16)
            for j in range(2):
                bw_s[j, t] = _dot_nt(p_phi, bqkv_in[:, j * D + c0:j * D + c1]).astype(BF16)
        bw_s[2] = bqkv_in[:, 2 * D:3 * D].T.reshape(n_slab, SW, D)
        bwo_s[...] = _pack(bwo_in[...])

    def project_ahead(first):
        def body(p, c):
            pl.when(first)(functools.partial(arrive, p))
            prefetch(p, first)
            xa = _unpack(xa_s[...])
            wo_s[p] = _pack(w_in[p, 3])
            for j, direct in ((2, 1), (0, 0), (1, 0)):
                w = w_in[p, j].T
                wqkv_s[p, :, j * PW:(j + 1) * PW] = _pack(w)
                n = min(PW, AHEAD - j * PW)
                if n > 0:
                    y = _dot_nt(xa, w_in[p, j, 0:n]) if direct else _dot(xa, w[:, 0:n])
                    ahead_s[p, :, :, j * PW:j * PW + n] = y.reshape(n_seg, SUB, n)
            return c

        lax.fori_loop(0, n_pair, body, 0)

    def block_diag(t):
        first = _iota((L, PW), 1) < dh
        return jnp.concatenate(
            [jnp.where(first, t, 0.0), jnp.where(first, 0.0, t)], axis=0).astype(BF16)

    def norm_for_b(s):
        xnb[s] = _pack(_layernorm(xres[s]).astype(BF16))

    def project_values(block, t):
        tokens = UNROLL * seg
        xn = _unpack(xnb[pl.ds(block * UNROLL, UNROLL)].reshape(tokens // 2, D))
        cols = pl.ds(pl.multiple_of(block * tokens, tokens), tokens)
        v = _dot_nt(bw_s[2, t], xn)
        for i in range(per_slab):
            v1 = jnp.concatenate([v[i * GW:(i + 1) * GW], jnp.ones((SUB, tokens), F32)], axis=0)
            v_s[t * per_slab + i, :, cols] = _pack(v1.astype(BF16))

    def a_step(s, mem, xn):
        h_full = jnp.concatenate([xn, mem], axis=0)
        h_rest = jnp.concatenate([xn[SUB:], mem], axis=0).astype(BF16)
        qi = _iota((L, 2 * L), 0)
        lane = _iota((L, 2 * L), 1)
        head_a = lane < L
        kj = jnp.where(head_a, lane, lane - L)
        visible = jnp.logical_or(qi < M, qi >= kj)

        def project(p):
            def rest():
                y = _dot(h_rest, _unpack(wqkv_s[p, :, 0:AHEAD]))
                return jnp.concatenate([y[-M:], ahead_s[p, s], y[:-M]], axis=0)

            def full():
                z = _dot(h_full, _unpack(wqkv_s[p, :, AHEAD:]))
                return jnp.concatenate([z[-M:], z[:-M]], axis=0)

            if AHEAD == 3 * PW:
                qkv = rest()
            elif 1:
                z = full()
                qkv = jnp.concatenate([rest(), z], axis=1)
            else:
                qkv = jnp.concatenate([rest(), full()], axis=1)
            return qkv[:, 0:PW], block_diag(qkv[:, PW:2 * PW]), block_diag(qkv[:, 2 * PW:])

        def probs(q, k):
            sc = jnp.where(visible, _dot_nt(q, k) * scale, -1e9)
            ma = jnp.max(jnp.where(head_a, sc, -jnp.inf), axis=-1, keepdims=True)
            mb = jnp.max(jnp.where(head_a, -jnp.inf, sc), axis=-1, keepdims=True)
            e = jnp.exp(sc - jnp.where(head_a, ma, mb))
            la = jnp.sum(jnp.where(head_a, e, 0.0), axis=-1, keepdims=True)
            lb = jnp.sum(jnp.where(head_a, 0.0, e), axis=-1, keepdims=True)
            return e / jnp.where(head_a, la, lb)

        norm_for_b(jnp.maximum(s - 1, 0))
        x_next = _layernorm(xres[jnp.minimum(s + 1, n_seg - 1)])

        lag_s, lag_v, lag_o = (1, 4, 6)
        qkv, pr, o = {}, {}, {}
        acc = None
        for t in range(n_pair + lag_o):
            if t < n_pair:
                qkv[t] = project(t)
            if 0 <= t - lag_s < n_pair:
                p = t - lag_s
                pr[p] = probs(qkv[p][0], qkv[p][1])
            if 0 <= t - lag_v < n_pair:
                p = t - lag_v
                o[p] = _dot(pr.pop(p), qkv.pop(p)[2])
            if 0 <= t - lag_o < n_pair:
                p = t - lag_o
                y = _dot(o.pop(p), _unpack(wo_s[p]))
                acc = y if acc is None else acc + y

        xres[s] = (xres[s].astype(F32) + acc[M:L]).astype(BF16)
        return acc[0:M], x_next

    def a_block(i, c):
        mem, xn = h_s[0:M], h_s[M:L]
        for u in range(UNROLL):
            mem, xn = a_step(i * UNROLL + u, mem, xn)
            project_values(jnp.maximum(i - 1, 0), u)
        h_s[0:M] = mem
        h_s[M:L] = xn
        return c

    def layer_a():
        h_s[0:M] = mem0_in[...].astype(F32)
        h_s[M:L] = _layernorm(xres[0])
        lax.fori_loop(0, n_seg // UNROLL, a_block, 0)
        norm_for_b(n_seg - 1)
        for t in range(n_slab):
            project_values(n_seg // UNROLL - 1, t)

    def b_keys(c, carry):
        n = CHUNK // seg
        xn = _unpack(xnb[pl.ds(c * n, n)].reshape(CHUNK // 2, D))
        cols = pl.ds(pl.multiple_of(c * CHUNK, CHUNK), CHUNK)

        def features(j, t):
            y = _dot_nt(bw_s[j, t], xn)
            return [_feature_map(y[i * GW:(i + 1) * GW]) for i in range(per_slab)]

        phi_k = []
        for t in range(n_slab):
            phi_k += features(1, t)
        for t in range(n_slab):
            for i, phi in enumerate(features(0, t)):
                phiq_s[t * per_slab + i, :, cols] = _pack(phi)
        for g in range(n_group):
            kv_s[g] += _dot_nt(_unpack(v_s[g, :, cols]), phi_k[g])
        return carry

    def out_cp(c):
        n = OUT_CHUNK // seg
        return pltpu.make_async_copy(
            xres.at[pl.ds(c * n, n)], out_hbm.at[pl.ds(c * n, n)], osem.at[c])

    def b_outputs(c, last):
        def attend(u):
            cols = pl.ds(pl.multiple_of(c * OUT_CHUNK + u * OUT_SUB, OUT_SUB), OUT_SUB)
            low = _iota((SUB, OUT_SUB), 0) < SUB // 2
            o = []
            for g in range(n_group):
                nd = _dot(kvm_s[g], _unpack(phiq_s[g, :, cols]))
                inv = 1.0 / (nd[GW:GW + SUB] + 1e-6)
                swapped = pltpu.roll(inv, SUB // 2, 0)
                head0, head1 = jnp.where(low, inv, swapped), jnp.where(low, swapped, inv)
                for i in range(0, GW, SUB):
                    w = head0 if i + SUB <= bd else head1 if i >= bd else inv
                    o.append(nd[i:i + SUB] * w)
            return jnp.concatenate(o, axis=0).astype(BF16)

        def finish(u, o_t):
            n = OUT_SUB // seg
            seg0 = c * (OUT_CHUNK // seg) + u * n
            y = _dot_tn(o_t, _unpack(bwo_s[...])).reshape(n, seg, D)
            y = (xres[pl.ds(seg0, n)].astype(F32) + y).astype(BF16)
            xres[pl.ds(seg0, n)] = y
            xa = _layernorm(y.astype(F32)[:, 0:SUB].reshape(n * SUB, D))
            xa_s[pl.ds(pl.multiple_of(seg0 * SUB // 2, n * SUB // 2), n * SUB // 2)] = (
                _pack(xa.astype(BF16)))

        n_sub = OUT_CHUNK // OUT_SUB
        o_t = attend(0)
        for u in range(n_sub):
            nxt = attend(u + 1) if u + 1 < n_sub else None
            finish(u, o_t)
            o_t = nxt

        @pl.when(last)
        def _():
            out_cp(c).start()

        return last

    def layer_b(last):
        kv_s[...] = jnp.zeros(kv_s.shape, F32)
        lax.fori_loop(0, S // CHUNK, b_keys, 0)
        shape = kv_s.shape[1:]
        r = _iota(shape, 0)
        row_head = jnp.where(r < GW, r // bd, (r - GW) // (SUB // GROUP))
        same_head = row_head == _iota(shape, 1) % GROUP
        for g in range(n_group):
            kvm_s[g] = jnp.where(same_head, kv_s[g], 0.0).astype(BF16)

        def body(c, carry):
            b_outputs(c, last)
            return carry

        lax.fori_loop(0, S // OUT_CHUNK, body, 0)

    def layer_pair(i, c):
        project_ahead(i == 0)
        pl.when(i == 0)(prepare_b)
        layer_a()
        layer_b(i == 1)
        return c

    begin()
    lax.fori_loop(0, 2, layer_pair, 0)
    for c in range(S // OUT_CHUNK):
        out_cp(c).wait()


@functools.partial(jax.jit, static_argnames=("A_seg_len",))
def pallas_interleave_layers__memory_aug_recurrent_mem_tr__linear_kernel_hedgehog__prompt_kernel(
    A_x: jax.Array,
    A_mem0: jax.Array,
    A_Wq: jax.Array,
    A_Wk: jax.Array,
    A_Wv: jax.Array,
    A_Wo: jax.Array,
    A_seg_len: int,
    B_x: jax.Array,
    B_wqkv: jax.Array,
    B_w_phi: jax.Array,
    B_wo: jax.Array,
):
    del B_x
    batch, S, D = A_x.shape
    _, H, dh = A_Wq.shape
    M = A_mem0.shape[1]
    seg = int(A_seg_len)
    n_seg = S // seg
    n_pair = H // 2
    bd = D // B_HEADS
    SW, GW = SLAB * bd, GROUP * bd
    n_group, n_slab = B_HEADS // GROUP, B_HEADS // SLAB
    assert batch == 1 and S % seg == 0 and S % CHUNK == 0 and S % OUT_CHUNK == 0 and H % 2 == 0
    assert UNROLL == n_slab and bd % SUB == SUB // 2 and A_x.dtype == BF16

    def head_major(w):
        return jnp.transpose(w, (1, 2, 0)).reshape(n_pair, 2 * dh, D)

    out = pl.pallas_call(
        functools.partial(_kernel, heads=H, dh=dh),
        out_shape=jax.ShapeDtypeStruct((n_seg, seg, D), BF16),
        in_specs=[pl.BlockSpec(memory_space=pl.ANY)] * 9,
        out_specs=pl.BlockSpec(memory_space=pl.ANY),
        scratch_shapes=[
            pltpu.VMEM((n_seg, seg, D), BF16),
            pltpu.VMEM((n_pair, D // 2, 6 * dh), U32),
            pltpu.VMEM((n_pair, dh, D), U32),
            pltpu.VMEM((n_pair, n_seg, SUB, AHEAD), F32),
            pltpu.VMEM((n_seg * SUB // 2, D), U32),
            pltpu.VMEM((n_seg, seg // 2, D), U32),
            pltpu.VMEM((3, n_slab, SW, D), BF16),
            pltpu.VMEM((D // 2, D), U32),
            pltpu.VMEM((n_group, (GW + SUB) // 2, S), U32),
            pltpu.VMEM((n_group, GW, S), U32),
            pltpu.VMEM((n_group, GW + SUB, 2 * GW), F32),
            pltpu.VMEM((n_group, GW + SUB, 2 * GW), BF16),
            pltpu.VMEM((M + seg, D), F32),
            pltpu.VMEM((n_pair, 4, 2 * dh, D), BF16),
            pltpu.VMEM((n_seg, SUB, D), BF16),
            pltpu.VMEM((M, D), BF16),
            pltpu.VMEM((D, 3 * D), BF16),
            pltpu.VMEM((bd, bd, B_HEADS), BF16),
            pltpu.VMEM((D, D), BF16),
            pltpu.VMEM((SW, D), F32),
            pltpu.SemaphoreType.DMA((n_pair, 4)),
            pltpu.SemaphoreType.DMA((6,)),
            pltpu.SemaphoreType.DMA((S // OUT_CHUNK,)),
        ],
        compiler_params=pltpu.CompilerParams(vmem_limit_bytes=126 * 1024 * 1024,
            disable_bounds_checks=bool(1)),
    )(
        A_x.reshape(n_seg, seg, D),
        A_mem0.reshape(M, D),
        head_major(A_Wq),
        head_major(A_Wk),
        head_major(A_Wv),
        A_Wo.reshape(n_pair, 2 * dh, D),
        B_wqkv,
        jnp.transpose(B_w_phi, (1, 2, 0)),
        B_wo,
    )
    return out.reshape(A_x.shape)
```

```python
import functools

import jax
import jax.numpy as jnp
from jax import lax
from jax.experimental import pallas as pl
from jax.experimental.pallas import tpu as pltpu

F32 = jnp.float32
BF16 = jnp.bfloat16
U32 = jnp.uint32

SUB = 8
B_HEADS = 32
GROUP = 2
SLAB = 8
UNROLL = 4
AHEAD = 7 * 128
IN_FLIGHT = 3
CHUNK = 512
OUT_CHUNK = 1024
OUT_SUB = 256

_NT = (((1,), (1,)), ((), ()))
_TN = (((0,), (0,)), ((), ()))


def _dot(a, b):
    return jnp.dot(a, b, preferred_element_type=F32)


def _dot_nt(a, b):
    return lax.dot_general(a, b, _NT, preferred_element_type=F32)


def _dot_tn(a, b):
    return lax.dot_general(a, b, _TN, preferred_element_type=F32)


def _pack(w):
    return pltpu.bitcast(w, U32)


def _unpack(w):
    return pltpu.bitcast(w, BF16)


def _layernorm(x):
    x = x.astype(F32)
    m = jnp.mean(x, axis=-1, keepdims=True)
    c = x - m
    v = jnp.mean(c * c, axis=-1, keepdims=True)
    return c * lax.rsqrt(v + 1e-5)


def _iota(shape, dim):
    return lax.broadcasted_iota(jnp.int32, shape, dim)


def _over_features(op, rows):
    r = functools.reduce(op, rows)
    shift = SUB // 2
    while shift >= GROUP:
        r = op(r, pltpu.roll(r, shift, 0))
        shift //= 2
    return r


def _feature_map(p):
    rows = [p[i:i + SUB] for i in range(0, p.shape[0], SUB)]
    hi = _over_features(jnp.maximum, rows)
    lo = _over_features(jnp.minimum, rows)
    ep = [jnp.exp(r - hi) for r in rows]
    en = [jnp.exp(lo - r) for r in rows]
    ip = 1.0 / _over_features(jnp.add, ep)
    im = 1.0 / _over_features(jnp.add, en)
    return jnp.concatenate([e * ip for e in ep] + [e * im for e in en], axis=0).astype(BF16)


def _kernel(x_hbm, mem0_hbm, wq_hbm, wk_hbm, wv_hbm, wo_hbm, bqkv_hbm, wphi_hbm, bwo_hbm,
            out_hbm,
            xres, wqkv_s, wo_s, ahead_s, xa_s, xnb, bw_s, bv_s, bwo_s, v_s, phiq_s, kv_s, kvm_s, h_s,
            w_in, xa_in, mem0_in, bqk_in, bv_in, wphi_in, bwo_in, phi_s, wsem, sem, osem,
            *, heads, dh):
    n_seg, seg, D = xres.shape
    S = n_seg * seg
    M = mem0_in.shape[0]
    L = M + seg
    n_pair = heads // 2
    PW = 2 * dh
    bd = D // B_HEADS
    GW = GROUP * bd
    SW = SLAB * bd
    n_group = B_HEADS // GROUP
    n_slab = B_HEADS // SLAB
    per_slab = SLAB // GROUP
    scale = dh ** -0.5

    xa_cp = pltpu.make_async_copy(x_hbm.at[:, 0:SUB], xa_in, sem.at[0])
    wphi_cp = pltpu.make_async_copy(wphi_hbm, wphi_in, sem.at[1])
    mem0_cp = pltpu.make_async_copy(mem0_hbm, mem0_in, sem.at[2])
    x_cp = pltpu.make_async_copy(x_hbm, xres, sem.at[3])
    bqk_cp = pltpu.make_async_copy(bqkv_hbm.at[:, 0:2 * D], bqk_in, sem.at[4])
    bv_cp = pltpu.make_async_copy(bqkv_hbm.at[:, 2 * D:3 * D], bv_in, sem.at[6])
    bwo_cp = pltpu.make_async_copy(bwo_hbm, bwo_in, sem.at[5])

    def w_cp(j, p):
        src = (wq_hbm, wk_hbm, wv_hbm, wo_hbm)[j]
        return pltpu.make_async_copy(src.at[p], w_in.at[p, j], wsem.at[p, j])

    def fetch(p):
        for j in range(4):
            w_cp(j, p).start()

    def begin():
        wphi_cp.start()
        xa_cp.start()
        xnb[0:UNROLL] = jnp.zeros((UNROLL,) + xnb.shape[1:], U32)
        wphi_cp.wait()
        fetch(0)
        col = _iota((B_HEADS, D), 1) - bd * _iota((B_HEADS, D), 0)
        phi_t = jnp.zeros((bd, D), F32)
        for d in range(bd):
            phi_t = phi_t + _dot(wphi_in[d], jnp.where(col == d, 1.0, 0.0).astype(BF16))
        row = _iota((SW, 128), 0) % GW
        spread = jnp.where(row // GROUP == _iota((SW, 128), 1), 1.0, 0.0)[:, 0:bd]
        phi_s[...] = _dot(spread, phi_t)
        xa_cp.wait()
        xa = xa_in[...].astype(F32).reshape(n_seg * SUB, D)
        xa_s[...] = _pack(_layernorm(xa).astype(BF16))
        for p in range(1, IN_FLIGHT):
            fetch(p)

    def arrive(p):
        for j in range(4):
            w_cp(j, p).wait()

    def prefetch(p, first):
        @pl.when(jnp.logical_and(first, p + IN_FLIGHT < n_pair))
        def _():
            fetch(p + IN_FLIGHT)

        for at, cp in zip((13, 14, 14), (x_cp, bv_cp, mem0_cp)):
            pl.when(jnp.logical_and(first, p == at))(cp.start)

    def prepare_a():
        bqk_cp.start()
        bwo_cp.start()
        for cp in (mem0_cp, x_cp, bv_cp):
            cp.wait()
        bv_s[...] = bv_in[...].T.reshape(n_slab, SW, D)

    def prepare_b():
        bqk_cp.wait()
        bwo_cp.wait()
        for t in range(n_slab):
            c0 = t * SW // 128 * 128
            c1 = -(-(t + 1) * SW // 128) * 128
            r = _iota((SW, c1 - c0), 0)
            head = t * SLAB + r // GW * GROUP + r % GROUP
            off = _iota((SW, c1 - c0), 1) + c0 - bd * head
            own = jnp.logical_and(off >= 0, off < bd)
            p_phi = jnp.where(own, phi_s[:, c0:c1], 0.0).astype(BF16)
            for j in range(2):
                bw_s[j, t] = _dot_nt(p_phi, bqk_in[:, j * D + c0:j * D + c1]).astype(BF16)
        bwo_s[...] = _pack(bwo_in[...])

    def project_ahead(first):
        def body(p, c):
            pl.when(first)(functools.partial(arrive, p))
            prefetch(p, first)
            xa = _unpack(xa_s[...])
            wo_s[p] = _pack(w_in[p, 3])
            for j in range(3):
                w = w_in[p, j].T
                wqkv_s[p, :, j * PW:(j + 1) * PW] = _pack(w)
                n = min(PW, AHEAD - j * PW)
                if n > 0:
                    y = _dot(xa, w[:, 0:n]) if j else _dot_nt(xa, w_in[p, j, 0:n])
                    ahead_s[p, :, :, j * PW:j * PW + n] = y.reshape(n_seg, SUB, n)
            return c

        lax.fori_loop(0, n_pair, body, 0)

    def block_diag(t):
        first = _iota((L, PW), 1) < dh
        return jnp.concatenate(
            [jnp.where(first, t, 0.0), jnp.where(first, 0.0, t)], axis=0).astype(BF16)

    def norm_for_b(s):
        xnb[s] = _pack(_layernorm(xres[s]).astype(BF16))

    def project_values(block, t):
        tokens = UNROLL * seg
        xn = _unpack(xnb[pl.ds(block * UNROLL, UNROLL)].reshape(tokens // 2, D))
        cols = pl.ds(pl.multiple_of(block * tokens, tokens), tokens)
        k0 = D // 512 * 512
        v = _dot_nt(bv_s[t, :, 0:k0], xn[:, 0:k0])
        w = bv_s[t, :, k0:].astype(F32)
        for i in range(per_slab):
            y = v[i * GW:(i + 1) * GW] + _dot_nt(w[i * GW:(i + 1) * GW], xn[:, k0:])
            v1 = jnp.concatenate([y, jnp.ones((SUB, tokens), F32)], axis=0)
            v_s[t * per_slab + i, :, cols] = _pack(v1.astype(BF16))

    def a_step(s, mem, xn):
        h_full = jnp.concatenate([xn, mem], axis=0)
        h_rest = jnp.concatenate([xn[SUB:], mem], axis=0).astype(BF16)
        qi = _iota((L, 2 * L), 0)
        lane = _iota((L, 2 * L), 1)
        head_a = lane < L
        kj = jnp.where(head_a, lane, lane - L)
        visible = jnp.logical_or(qi < M, qi >= kj)

        def project(p):
            y = _dot(h_rest, _unpack(wqkv_s[p, :, 0:AHEAD]))
            z = _dot(h_full, _unpack(wqkv_s[p, :, AHEAD:]))
            qkv = jnp.concatenate([
                jnp.concatenate([y[-M:], ahead_s[p, s], y[:-M]], axis=0),
                jnp.concatenate([z[-M:], z[:-M]], axis=0)], axis=1)
            return qkv[:, 0:PW], block_diag(qkv[:, PW:2 * PW]), block_diag(qkv[:, 2 * PW:])

        def probs(q, k):
            sc = jnp.where(visible, _dot_nt(q, k) * scale, -1e9)
            ma = jnp.max(jnp.where(head_a, sc, -jnp.inf), axis=-1, keepdims=True)
            mb = jnp.max(jnp.where(head_a, -jnp.inf, sc), axis=-1, keepdims=True)
            e = jnp.exp(sc - jnp.where(head_a, ma, mb))
            la = jnp.sum(jnp.where(head_a, e, 0.0), axis=-1, keepdims=True)
            lb = jnp.sum(jnp.where(head_a, 0.0, e), axis=-1, keepdims=True)
            return e / jnp.where(head_a, la, lb)

        norm_for_b(jnp.maximum(s - 1, 0))
        x_next = _layernorm(xres[jnp.minimum(s + 1, n_seg - 1)])

        lag_s, lag_v, lag_o = (1, 4, 6)
        qkv, pr, o = {}, {}, {}
        acc = None
        for t in range(n_pair + lag_o):
            if t < n_pair:
                qkv[t] = project(t)
            if 0 <= t - lag_o < n_pair:
                p = t - lag_o
                y = _dot(o.pop(p), _unpack(wo_s[p]))
                acc = y if acc is None else acc + y
            if 0 <= t - lag_v < n_pair:
                p = t - lag_v
                o[p] = _dot(pr.pop(p), qkv.pop(p)[2])
            if 0 <= t - lag_s < n_pair:
                p = t - lag_s
                pr[p] = probs(qkv[p][0], qkv[p][1])

        xres[s] = (xres[s].astype(F32) + acc[M:L]).astype(BF16)
        return acc[0:M], x_next

    def a_block(i, c):
        mem, xn = h_s[0:M], h_s[M:L]
        for u in range(UNROLL):
            mem, xn = a_step(i * UNROLL + u, mem, xn)
            project_values(jnp.maximum(i - 1, 0), u)
        h_s[0:M] = mem
        h_s[M:L] = xn
        return c

    def layer_a():
        h_s[0:M] = mem0_in[...].astype(F32)
        h_s[M:L] = _layernorm(xres[0])
        lax.fori_loop(0, n_seg // UNROLL, a_block, 0)
        norm_for_b(n_seg - 1)
        for t in range(n_slab):
            project_values(n_seg // UNROLL - 1, t)

    def b_keys(c, carry):
        n = CHUNK // seg
        xn = _unpack(xnb[pl.ds(c * n, n)].reshape(CHUNK // 2, D))
        cols = pl.ds(pl.multiple_of(c * CHUNK, CHUNK), CHUNK)

        def features(j, t):
            y = _dot_nt(bw_s[j, t], xn)
            return [_feature_map(y[i * GW:(i + 1) * GW]) for i in range(per_slab)]

        phi_k = []
        for t in range(n_slab):
            phi_k += features(1, t)
        for t in range(n_slab):
            for i, phi in enumerate(features(0, t)):
                phiq_s[t * per_slab + i, :, cols] = _pack(phi)
        for g in range(n_group):
            kv_s[g] += _dot_nt(_unpack(v_s[g, :, cols]), phi_k[g])
        return carry

    def out_cp(c, tail=False):
        n, m = OUT_CHUNK // seg, OUT_SUB // seg
        rows = pl.ds(c * n + n - m, m) if tail else pl.ds(c * n, n - m)
        return pltpu.make_async_copy(xres.at[rows], out_hbm.at[rows], osem.at[c, int(tail)])

    def b_outputs(c, last):
        def attend(u):
            cols = pl.ds(pl.multiple_of(c * OUT_CHUNK + u * OUT_SUB, OUT_SUB), OUT_SUB)
            low = _iota((SUB, OUT_SUB), 0) < SUB // 2
            o = []
            for g in range(n_group):
                nd = _dot(kvm_s[g], _unpack(phiq_s[g, :, cols]))
                inv = 1.0 / (nd[GW:GW + SUB] + 1e-6)
                swapped = pltpu.roll(inv, SUB // 2, 0)
                head0, head1 = jnp.where(low, inv, swapped), jnp.where(low, swapped, inv)
                for i in range(0, GW, SUB):
                    w = head0 if i + SUB <= bd else head1 if i >= bd else inv
                    o.append(nd[i:i + SUB] * w)
            return jnp.concatenate(o, axis=0).astype(BF16)

        def finish(u, o_t):
            n = OUT_SUB // seg
            seg0 = c * (OUT_CHUNK // seg) + u * n
            y = _dot_tn(o_t, _unpack(bwo_s[...])).reshape(n, seg, D)
            y = (xres[pl.ds(seg0, n)].astype(F32) + y).astype(BF16)
            xres[pl.ds(seg0, n)] = y
            xa = _layernorm(y.astype(F32)[:, 0:SUB].reshape(n * SUB, D))
            xa_s[pl.ds(pl.multiple_of(seg0 * SUB // 2, n * SUB // 2), n * SUB // 2)] = (
                _pack(xa.astype(BF16)))

        n_sub = OUT_CHUNK // OUT_SUB
        o_t = attend(0)
        for u in range(n_sub):
            nxt = attend(u + 1) if u + 1 < n_sub else None
            finish(u, o_t)
            o_t = nxt
            if u == n_sub - 2:
                pl.when(last)(out_cp(c).start)

        pl.when(last)(out_cp(c, tail=True).start)

    def layer_b(last):
        kv_s[...] = jnp.zeros(kv_s.shape, F32)
        lax.fori_loop(0, S // CHUNK, b_keys, 0)
        shape = kv_s.shape[1:]
        r = _iota(shape, 0)
        row_head = jnp.where(r < GW, r // bd, (r - GW) // (SUB // GROUP))
        same_head = row_head == _iota(shape, 1) % GROUP
        for g in range(n_group):
            kvm_s[g] = jnp.where(same_head, kv_s[g], 0.0).astype(BF16)
        lax.fori_loop(0, S // OUT_CHUNK, lambda c, _: b_outputs(c, last), None)

    def layer_pair(i, c):
        project_ahead(i == 0)
        pl.when(i == 0)(prepare_a)
        layer_a()
        pl.when(i == 0)(prepare_b)
        layer_b(i == 1)
        return c

    begin()
    lax.fori_loop(0, 2, layer_pair, 0)
    for c in range(S // OUT_CHUNK):
        out_cp(c).wait()
        out_cp(c, tail=True).wait()


@functools.partial(jax.jit, static_argnames=("A_seg_len",))
def pallas_interleave_layers__memory_aug_recurrent_mem_tr__linear_kernel_hedgehog__prompt_kernel(
    A_x: jax.Array,
    A_mem0: jax.Array,
    A_Wq: jax.Array,
    A_Wk: jax.Array,
    A_Wv: jax.Array,
    A_Wo: jax.Array,
    A_seg_len: int,
    B_x: jax.Array,
    B_wqkv: jax.Array,
    B_w_phi: jax.Array,
    B_wo: jax.Array,
):
    del B_x
    batch, S, D = A_x.shape
    _, H, dh = A_Wq.shape
    M = A_mem0.shape[1]
    seg = int(A_seg_len)
    n_seg = S // seg
    n_pair = H // 2
    bd = D // B_HEADS
    SW, GW = SLAB * bd, GROUP * bd
    n_group, n_slab = B_HEADS // GROUP, B_HEADS // SLAB
    assert batch == 1 and S % seg == 0 and S % CHUNK == 0 and S % OUT_CHUNK == 0 and H % 2 == 0
    assert UNROLL == n_slab and bd % SUB == SUB // 2 and A_x.dtype == BF16

    def head_major(w):
        return jnp.transpose(w, (1, 2, 0)).reshape(n_pair, 2 * dh, D)

    out = pl.pallas_call(
        functools.partial(_kernel, heads=H, dh=dh),
        out_shape=jax.ShapeDtypeStruct((n_seg, seg, D), BF16),
        in_specs=[pl.BlockSpec(memory_space=pl.ANY)] * 9,
        out_specs=pl.BlockSpec(memory_space=pl.ANY),
        scratch_shapes=[
            pltpu.VMEM((n_seg, seg, D), BF16),
            pltpu.VMEM((n_pair, D // 2, 6 * dh), U32),
            pltpu.VMEM((n_pair, dh, D), U32),
            pltpu.VMEM((n_pair, n_seg, SUB, AHEAD), F32),
            pltpu.VMEM((n_seg * SUB // 2, D), U32),
            pltpu.VMEM((n_seg, seg // 2, D), U32),
            pltpu.VMEM((2, n_slab, SW, D), BF16),
            pltpu.VMEM((n_slab, SW, D), BF16),
            pltpu.VMEM((D // 2, D), U32),
            pltpu.VMEM((n_group, (GW + SUB) // 2, S), U32),
            pltpu.VMEM((n_group, GW, S), U32),
            pltpu.VMEM((n_group, GW + SUB, 2 * GW), F32),
            pltpu.VMEM((n_group, GW + SUB, 2 * GW), BF16),
            pltpu.VMEM((M + seg, D), F32),
            pltpu.VMEM((n_pair, 4, 2 * dh, D), BF16),
            pltpu.VMEM((n_seg, SUB, D), BF16),
            pltpu.VMEM((M, D), BF16),
            pltpu.VMEM((D, 2 * D), BF16),
            pltpu.VMEM((D, D), BF16),
            pltpu.VMEM((bd, bd, B_HEADS), BF16),
            pltpu.VMEM((D, D), BF16),
            pltpu.VMEM((SW, D), F32),
            pltpu.SemaphoreType.DMA((n_pair, 4)),
            pltpu.SemaphoreType.DMA((7,)),
            pltpu.SemaphoreType.DMA((S // OUT_CHUNK, 2)),
        ],
        compiler_params=pltpu.CompilerParams(vmem_limit_bytes=126 * 1024 * 1024,
            disable_bounds_checks=True),
    )(
        A_x.reshape(n_seg, seg, D),
        A_mem0.reshape(M, D),
        head_major(A_Wq),
        head_major(A_Wk),
        head_major(A_Wv),
        A_Wo.reshape(n_pair, 2 * dh, D),
        B_wqkv,
        jnp.transpose(B_w_phi, (1, 2, 0)),
        B_wo,
    )
    return out.reshape(A_x.shape)
```

```python
import functools

import jax
import jax.numpy as jnp
from jax import lax
from jax.experimental import pallas as pl
from jax.experimental.pallas import tpu as pltpu

F32 = jnp.float32
BF16 = jnp.bfloat16
U32 = jnp.uint32

SUB = 8
B_HEADS = 32
GROUP = 2
SLAB = 8
UNROLL = 4
AHEAD = 7 * 128
IN_FLIGHT = 3
CHUNK = 512
OUT_CHUNK = 1024
OUT_SUB = 256

_NT = (((1,), (1,)), ((), ()))
_TN = (((0,), (0,)), ((), ()))


def _dot(a, b):
    return jnp.dot(a, b, preferred_element_type=F32)


def _dot_nt(a, b):
    return lax.dot_general(a, b, _NT, preferred_element_type=F32)


def _dot_tn(a, b):
    return lax.dot_general(a, b, _TN, preferred_element_type=F32)


def _pack(w):
    return pltpu.bitcast(w, U32)


def _unpack(w):
    return pltpu.bitcast(w, BF16)


def _layernorm(x):
    x = x.astype(F32)
    m = jnp.mean(x, axis=-1, keepdims=True)
    c = x - m
    v = jnp.mean(c * c, axis=-1, keepdims=True)
    return c * lax.rsqrt(v + 1e-5)


def _iota(shape, dim):
    return lax.broadcasted_iota(jnp.int32, shape, dim)


def _over_features(op, rows):
    r = functools.reduce(op, rows)
    shift = SUB // 2
    while shift >= GROUP:
        r = op(r, pltpu.roll(r, shift, 0))
        shift //= 2
    return r


def _feature_map(p):
    rows = [p[i:i + SUB] for i in range(0, p.shape[0], SUB)]
    hi = _over_features(jnp.maximum, rows)
    lo = _over_features(jnp.minimum, rows)
    ep = [jnp.exp(r - hi) for r in rows]
    en = [jnp.exp(lo - r) for r in rows]
    ip = 1.0 / _over_features(jnp.add, ep)
    im = 1.0 / _over_features(jnp.add, en)
    return jnp.concatenate([e * ip for e in ep] + [e * im for e in en], axis=0).astype(BF16)


def _kernel(x_hbm, mem0_hbm, wq_hbm, wk_hbm, wv_hbm, wo_hbm, bqkv_hbm, wphi_hbm, bwo_hbm,
            out_hbm,
            xres, wqkv_s, wo_s, ahead_s, xa_s, xnb, bw_s, bv_s, bwo_s, v_s, phiq_s, kv_s, kvm_s, h_s,
            w_in, xa_in, mem0_in, bqk_in, bv_in, wphi_in, bwo_in, phi_s, wsem, sem, osem,
            *, heads, dh):
    n_seg, seg, D = xres.shape
    S = n_seg * seg
    M = mem0_in.shape[0]
    L = M + seg
    n_pair = heads // 2
    PW = 2 * dh
    bd = D // B_HEADS
    GW = GROUP * bd
    SW = SLAB * bd
    n_group = B_HEADS // GROUP
    n_slab = B_HEADS // SLAB
    per_slab = SLAB // GROUP
    scale = dh ** -0.5

    xa_cp = pltpu.make_async_copy(x_hbm.at[:, 0:SUB], xa_in, sem.at[0])
    wphi_cp = pltpu.make_async_copy(wphi_hbm, wphi_in, sem.at[1])
    mem0_cp = pltpu.make_async_copy(mem0_hbm, mem0_in, sem.at[2])
    x_cp = pltpu.make_async_copy(x_hbm, xres, sem.at[3])
    bqk_cp = pltpu.make_async_copy(bqkv_hbm.at[:, 0:2 * D], bqk_in, sem.at[4])
    bv_cp = pltpu.make_async_copy(bqkv_hbm.at[:, 2 * D:3 * D], bv_in, sem.at[6])
    bwo_cp = pltpu.make_async_copy(bwo_hbm, bwo_in, sem.at[5])

    def w_cp(j, p):
        src = (wq_hbm, wk_hbm, wv_hbm, wo_hbm)[j]
        return pltpu.make_async_copy(src.at[p], w_in.at[p, j], wsem.at[p, j])

    def fetch(p):
        for j in range(4):
            w_cp(j, p).start()

    def begin():
        wphi_cp.start()
        xa_cp.start()
        xnb[0:UNROLL] = jnp.zeros((UNROLL,) + xnb.shape[1:], U32)
        wphi_cp.wait()
        fetch(0)
        col = _iota((B_HEADS, D), 1) - bd * _iota((B_HEADS, D), 0)
        phi_t = jnp.zeros((bd, D), F32)
        for d in range(bd):
            phi_t = phi_t + _dot(wphi_in[d], jnp.where(col == d, 1.0, 0.0).astype(BF16))
        row = _iota((SW, 128), 0) % GW
        spread = jnp.where(row // GROUP == _iota((SW, 128), 1), 1.0, 0.0)[:, 0:bd]
        phi_s[...] = _dot(spread, phi_t)
        xa_cp.wait()
        xa = xa_in[...].astype(F32).reshape(n_seg * SUB, D)
        xa_s[...] = _pack(_layernorm(xa).astype(BF16))
        for p in range(1, IN_FLIGHT):
            fetch(p)

    def arrive(p):
        for j in range(4):
            w_cp(j, p).wait()

        @pl.when(p + IN_FLIGHT < n_pair)
        def _():
            fetch(p + IN_FLIGHT)

        @pl.when(p == n_pair - IN_FLIGHT)
        def _():
            for cp in (x_cp, bv_cp, mem0_cp):
                cp.start()

    def prepare_a():
        bqk_cp.start()
        bwo_cp.start()
        for cp in (mem0_cp, x_cp, bv_cp):
            cp.wait()
        bv_s[...] = bv_in[...].T.reshape(n_slab, SW, D)

    def prepare_b():
        bqk_cp.wait()
        bwo_cp.wait()
        n = SW // 2
        for r0 in range(0, D, n):
            c0, c1 = r0 // 128 * 128, -(-(r0 + n) // 128) * 128
            r = _iota((n, c1 - c0), 0) + r0
            off = _iota((n, c1 - c0), 1) + c0 - bd * (r // GW * GROUP + r % GROUP)
            own = jnp.logical_and(off >= 0, off < bd)
            p_phi = jnp.where(own, phi_s[0:n, c0:c1], 0.0).astype(BF16)
            for j in range(2):
                w = _dot_nt(p_phi, bqk_in[:, j * D + c0:j * D + c1])
                bw_s[j, r0 // SW, r0 % SW:r0 % SW + n] = w.astype(BF16)
        bwo_s[...] = _pack(bwo_in[...])

    def project_ahead(first):
        def body(p, c):
            pl.when(first)(functools.partial(arrive, p))
            xa = _unpack(xa_s[...])
            wo_s[p] = _pack(w_in[p, 3])
            for j in range(3):
                w = w_in[p, j].T
                wqkv_s[p, :, j * PW:(j + 1) * PW] = _pack(w)
                n = min(PW, AHEAD - j * PW)
                if n > 0:
                    y = _dot(xa, w[:, 0:n]) if j else _dot_nt(xa, w_in[p, j, 0:n])
                    ahead_s[p, :, :, j * PW:j * PW + n] = y.reshape(n_seg, SUB, n)
            return c

        lax.fori_loop(0, n_pair, body, 0)

    def block_diag(t):
        first = _iota((L, PW), 1) < dh
        return jnp.concatenate(
            [jnp.where(first, t, 0.0), jnp.where(first, 0.0, t)], axis=0).astype(BF16)

    def norm_for_b(s):
        xnb[s] = _pack(_layernorm(xres[s]).astype(BF16))

    def project_values(block, t):
        tokens = UNROLL * seg
        xn = _unpack(xnb[pl.ds(block * UNROLL, UNROLL)].reshape(tokens // 2, D))
        cols = pl.ds(pl.multiple_of(block * tokens, tokens), tokens)
        k0 = D // 512 * 512
        v = _dot_nt(bv_s[t, :, 0:k0], xn[:, 0:k0])
        w = bv_s[t, :, k0:].astype(F32)
        for i in range(per_slab):
            y = v[i * GW:(i + 1) * GW] + _dot_nt(w[i * GW:(i + 1) * GW], xn[:, k0:])
            v1 = jnp.concatenate([y, jnp.ones((SUB, tokens), F32)], axis=0)
            v_s[t * per_slab + i, :, cols] = _pack(v1.astype(BF16))

    def a_step(s, mem, xn):
        h_full = jnp.concatenate([xn, mem], axis=0)
        h_rest = jnp.concatenate([xn[SUB:], mem], axis=0).astype(BF16)
        qi = _iota((L, 2 * L), 0)
        lane = _iota((L, 2 * L), 1)
        head_a = lane < L
        kj = jnp.where(head_a, lane, lane - L)
        visible = jnp.logical_or(qi < M, qi >= kj)

        def project(p):
            y = _dot(h_rest, _unpack(wqkv_s[p, :, 0:AHEAD]))
            z = _dot(h_full, _unpack(wqkv_s[p, :, AHEAD:]))
            qkv = jnp.concatenate([
                jnp.concatenate([y[-M:], ahead_s[p, s], y[:-M]], axis=0),
                jnp.concatenate([z[-M:], z[:-M]], axis=0)], axis=1)
            return qkv[:, 0:PW], block_diag(qkv[:, PW:2 * PW]), block_diag(qkv[:, 2 * PW:])

        def probs(q, k):
            sc = jnp.where(visible, _dot_nt(q, k) * scale, -1e9)
            ma = jnp.max(jnp.where(head_a, sc, -jnp.inf), axis=-1, keepdims=True)
            mb = jnp.max(jnp.where(head_a, -jnp.inf, sc), axis=-1, keepdims=True)
            e = jnp.exp(sc - jnp.where(head_a, ma, mb))
            la = jnp.sum(jnp.where(head_a, e, 0.0), axis=-1, keepdims=True)
            lb = jnp.sum(jnp.where(head_a, 0.0, e), axis=-1, keepdims=True)
            return e / jnp.where(head_a, la, lb)

        norm_for_b(jnp.maximum(s - 1, 0))
        x_next = _layernorm(xres[jnp.minimum(s + 1, n_seg - 1)])

        lag_s, lag_v, lag_o = (1, 4, 6)
        qkv, pr, o = {}, {}, {}
        acc = None
        for t in range(n_pair + lag_o):
            if t < n_pair:
                qkv[t] = project(t)
            if 0 <= t - lag_o < n_pair:
                p = t - lag_o
                y = _dot(o.pop(p), _unpack(wo_s[p]))
                acc = y if acc is None else acc + y
            if 0 <= t - lag_v < n_pair:
                p = t - lag_v
                o[p] = _dot(pr.pop(p), qkv.pop(p)[2])
            if 0 <= t - lag_s < n_pair:
                p = t - lag_s
                pr[p] = probs(qkv[p][0], qkv[p][1])

        xres[s] = (xres[s].astype(F32) + acc[M:L]).astype(BF16)
        return acc[0:M], x_next

    def a_block(i, c):
        mem, xn = h_s[0:M], h_s[M:L]
        for u in range(UNROLL):
            mem, xn = a_step(i * UNROLL + u, mem, xn)
            project_values(jnp.maximum(i - 1, 0), u)
        h_s[0:M] = mem
        h_s[M:L] = xn
        return c

    def layer_a():
        h_s[0:M] = mem0_in[...].astype(F32)
        h_s[M:L] = _layernorm(xres[0])
        lax.fori_loop(0, n_seg // UNROLL, a_block, 0)
        norm_for_b(n_seg - 1)
        for t in range(n_slab):
            project_values(n_seg // UNROLL - 1, t)

    def b_keys(c, carry):
        n = CHUNK // seg
        xn = _unpack(xnb[pl.ds(c * n, n)].reshape(CHUNK // 2, D))
        cols = pl.ds(pl.multiple_of(c * CHUNK, CHUNK), CHUNK)

        def features(j, t):
            y = _dot_nt(bw_s[j, t], xn)
            return [_feature_map(y[i * GW:(i + 1) * GW]) for i in range(per_slab)]

        phi_k = []
        for t in range(n_slab):
            phi_k += features(1, t)
        for t in range(n_slab):
            for i, phi in enumerate(features(0, t)):
                phiq_s[t * per_slab + i, :, cols] = _pack(phi)
        for g in range(n_group):
            kv_s[g] += _dot_nt(_unpack(v_s[g, :, cols]), phi_k[g])
        return carry

    def out_cp(c, tail=False):
        n, m = OUT_CHUNK // seg, OUT_SUB // seg
        rows = pl.ds(c * n + n - m, m) if tail else pl.ds(c * n, n - m)
        return pltpu.make_async_copy(xres.at[rows], out_hbm.at[rows], osem.at[c, int(tail)])

    def b_outputs(c, last):
        def attend(u):
            cols = pl.ds(pl.multiple_of(c * OUT_CHUNK + u * OUT_SUB, OUT_SUB), OUT_SUB)
            low = _iota((SUB, OUT_SUB), 0) < SUB // 2
            o = []
            for g in range(n_group):
                nd = _dot(kvm_s[g], _unpack(phiq_s[g, :, cols]))
                inv = 1.0 / (nd[GW:GW + SUB] + 1e-6)
                swapped = pltpu.roll(inv, SUB // 2, 0)
                head0, head1 = jnp.where(low, inv, swapped), jnp.where(low, swapped, inv)
                for i in range(0, GW, SUB):
                    w = head0 if i + SUB <= bd else head1 if i >= bd else inv
                    o.append(nd[i:i + SUB] * w)
            return jnp.concatenate(o, axis=0).astype(BF16)

        def finish(u, o_t):
            n = OUT_SUB // seg
            seg0 = c * (OUT_CHUNK // seg) + u * n
            y = _dot_tn(o_t, _unpack(bwo_s[...])).reshape(n, seg, D)
            y = (xres[pl.ds(seg0, n)].astype(F32) + y).astype(BF16)
            xres[pl.ds(seg0, n)] = y
            xa = _layernorm(y.astype(F32)[:, 0:SUB].reshape(n * SUB, D))
            xa_s[pl.ds(pl.multiple_of(seg0 * SUB // 2, n * SUB // 2), n * SUB // 2)] = (
                _pack(xa.astype(BF16)))

        n_sub = OUT_CHUNK // OUT_SUB
        lead = 3
        o_t = {}
        for t in range(n_sub + lead):
            if t < n_sub:
                o_t[t] = attend(t)
            if t >= lead:
                finish(t - lead, o_t.pop(t - lead))
            if t - lead == n_sub - 2:
                pl.when(last)(out_cp(c).start)
        pl.when(last)(out_cp(c, tail=True).start)

    def layer_b(last):
        kv_s[...] = jnp.zeros(kv_s.shape, F32)
        lax.fori_loop(0, S // CHUNK, b_keys, 0)
        shape = kv_s.shape[1:]
        r = _iota(shape, 0)
        row_head = jnp.where(r < GW, r // bd, (r - GW) // (SUB // GROUP))
        same_head = row_head == _iota(shape, 1) % GROUP
        for g in range(n_group):
            kvm_s[g] = jnp.where(same_head, kv_s[g], 0.0).astype(BF16)
        lax.fori_loop(0, S // OUT_CHUNK, lambda c, _: b_outputs(c, last), None)

    def layer_pair(i, c):
        project_ahead(i == 0)
        pl.when(i == 0)(prepare_a)
        layer_a()
        pl.when(i == 0)(prepare_b)
        layer_b(i == 1)
        return c

    begin()
    lax.fori_loop(0, 2, layer_pair, 0)
    for c in range(S // OUT_CHUNK):
        out_cp(c).wait()
        out_cp(c, tail=True).wait()


@functools.partial(jax.jit, static_argnames=("A_seg_len",))
def pallas_interleave_layers__memory_aug_recurrent_mem_tr__linear_kernel_hedgehog__prompt_kernel(
    A_x: jax.Array,
    A_mem0: jax.Array,
    A_Wq: jax.Array,
    A_Wk: jax.Array,
    A_Wv: jax.Array,
    A_Wo: jax.Array,
    A_seg_len: int,
    B_x: jax.Array,
    B_wqkv: jax.Array,
    B_w_phi: jax.Array,
    B_wo: jax.Array,
):
    del B_x
    batch, S, D = A_x.shape
    _, H, dh = A_Wq.shape
    M = A_mem0.shape[1]
    seg = int(A_seg_len)
    n_seg = S // seg
    n_pair = H // 2
    bd = D // B_HEADS
    SW, GW = SLAB * bd, GROUP * bd
    n_group, n_slab = B_HEADS // GROUP, B_HEADS // SLAB
    assert batch == 1 and S % seg == 0 and S % CHUNK == 0 and S % OUT_CHUNK == 0 and H % 2 == 0
    assert UNROLL == n_slab and bd % SUB == SUB // 2 and A_x.dtype == BF16

    def head_major(w):
        return jnp.transpose(w, (1, 2, 0)).reshape(n_pair, 2 * dh, D)

    out = pl.pallas_call(
        functools.partial(_kernel, heads=H, dh=dh),
        out_shape=jax.ShapeDtypeStruct((n_seg, seg, D), BF16),
        in_specs=[pl.BlockSpec(memory_space=pl.ANY)] * 9,
        out_specs=pl.BlockSpec(memory_space=pl.ANY),
        scratch_shapes=[
            pltpu.VMEM((n_seg, seg, D), BF16),
            pltpu.VMEM((n_pair, D // 2, 6 * dh), U32),
            pltpu.VMEM((n_pair, dh, D), U32),
            pltpu.VMEM((n_pair, n_seg, SUB, AHEAD), F32),
            pltpu.VMEM((n_seg * SUB // 2, D), U32),
            pltpu.VMEM((n_seg, seg // 2, D), U32),
            pltpu.VMEM((2, n_slab, SW, D), BF16),
            pltpu.VMEM((n_slab, SW, D), BF16),
            pltpu.VMEM((D // 2, D), U32),
            pltpu.VMEM((n_group, (GW + SUB) // 2, S), U32),
            pltpu.VMEM((n_group, GW, S), U32),
            pltpu.VMEM((n_group, GW + SUB, 2 * GW), F32),
            pltpu.VMEM((n_group, GW + SUB, 2 * GW), BF16),
            pltpu.VMEM((M + seg, D), F32),
            pltpu.VMEM((n_pair, 4, 2 * dh, D), BF16),
            pltpu.VMEM((n_seg, SUB, D), BF16),
            pltpu.VMEM((M, D), BF16),
            pltpu.VMEM((D, 2 * D), BF16),
            pltpu.VMEM((D, D), BF16),
            pltpu.VMEM((bd, bd, B_HEADS), BF16),
            pltpu.VMEM((D, D), BF16),
            pltpu.VMEM((SW, D), F32),
            pltpu.SemaphoreType.DMA((n_pair, 4)),
            pltpu.SemaphoreType.DMA((7,)),
            pltpu.SemaphoreType.DMA((S // OUT_CHUNK, 2)),
        ],
        compiler_params=pltpu.CompilerParams(vmem_limit_bytes=126 * 1024 * 1024,
            disable_bounds_checks=True),
    )(
        A_x.reshape(n_seg, seg, D),
        A_mem0.reshape(M, D),
        head_major(A_Wq),
        head_major(A_Wk),
        head_major(A_Wv),
        A_Wo.reshape(n_pair, 2 * dh, D),
        B_wqkv,
        jnp.transpose(B_w_phi, (1, 2, 0)),
        B_wo,
    )
    return out.reshape(A_x.shape)
```
